```python
import os as _os
_os.environ.setdefault("JAX_PLATFORMS", "cpu")
import jax
import jax.numpy as jnp

def _softmax(x, axis=-1):
    return jax.nn.softmax(x, axis=axis)
def _gelu(x):
    return jax.nn.gelu(x, approximate=True)
def _silu(x):
    return jax.nn.silu(x)
def _sigmoid(x):
    return jax.nn.sigmoid(x)
def _layernorm(x, axis=-1, eps=1e-5):
    m = jnp.mean(x, axis=axis, keepdims=True)
    v = jnp.var(x, axis=axis, keepdims=True)
    return (x - m) / jnp.sqrt(v + eps)
def _scatter_add(tgt, idx, src, axis=0):
    return tgt.at[idx].add(src)
def _segment_sum(src, seg, n):
    return jax.ops.segment_sum(src, seg, n)
class _Rng:
    def __init__(self, key):
        self._k = key
    def _next(self):
        self._k, sub = jax.random.split(self._k)
        return sub
    def normal(self, shape):
        return jax.random.normal(self._next(), shape, dtype=jnp.bfloat16)
    def randint(self, lo, hi, shape):
        return jax.random.randint(self._next(), shape, lo, hi, dtype=jnp.int32)
    def uniform(self, shape, lo=0.0, hi=1.0):
        return jax.random.uniform(self._next(), shape, jnp.bfloat16, lo, hi)
    def permutation(self, n):
        return jax.random.permutation(self._next(), n)


kernel_name = 'gated_mix__sliding_local_dilated__moe_arch_mod__prompt'

def setup_inputs():
    _rng = _Rng(jax.random.key(int.from_bytes(__import__("os").urandom(4), "little")))
    _w = (lambda a: (lambda t: t.astype(jnp.bfloat16) if jnp.issubdtype(t.dtype, jnp.floating) else t)(jnp.asarray(a)))
    def _A_setup():
        B, S, D = 1, 2048, 640
        return {
            "x": _w((lambda *s: _rng.normal(s) * 0.05)(B, S, D)),
            "wqkv": _w((lambda *s: _rng.normal(s) * 0.8)(D, 3 * D)),
            "wo": _w((lambda *s: _rng.normal(s) * 0.05)(D, D)),
        }
    _A_in = _A_setup()

    def _B_setup():
        B, S, D, F, C = 1, 2048, 640, 1728, 1
        return {
            "x": _w((lambda *s: _rng.normal(s) * 0.05)(B, S, D)),
            "w_r": _w((lambda *s: _rng.normal(s) * 1.6)(D)),
            "w_gate": _w((lambda *s: _rng.normal(s) * 0.4)(D, F)),
            "w_up": _w((lambda *s: _rng.normal(s) * 0.4)(D, F)),
            "w_down": _w((lambda *s: _rng.normal(s) * 0.4)(F, D)),
        }
    _B_in = _B_setup()

    return {
        "A_x": _A_in["x"],
        "A_wqkv": _A_in["wqkv"],
        "A_wo": _A_in["wo"],
        "B_x": _B_in["x"],
        "B_w_r": _B_in["w_r"],
        "B_w_gate": _B_in["w_gate"],
        "B_w_up": _B_in["w_up"],
        "B_w_down": _B_in["w_down"],
        "gate_w": _w((lambda *s: _rng.normal(s) * 0.05)(640) * 16.0),
    }

def reference(A_x, A_wqkv, A_wo, B_x, B_w_r, B_w_gate, B_w_up, B_w_down, gate_w):
    def _A_ref(x, wqkv, wo):
        B, S, D = x.shape
        H = 32; Dh = D // H
        W, dil = 8, 2
        qkv = (lambda x, *d: x.transpose(*d))((x @ wqkv).reshape(B, S, 3, H, Dh), 2, 0, 3, 1, 4)
        q, k, v = qkv[0], qkv[1], qkv[2]
        scale = Dh ** -0.5
        pos = jnp.arange(S)
        off = jnp.arange(W) * dil
        idx = pos[:, None] - off[None, :]
        mask = idx >= 0
        idx_c = jnp.where(mask, idx, 0).reshape(-1)
        kg = k[:, :, idx_c, :].reshape(B, H, S, W, Dh)
        vg = v[:, :, idx_c, :].reshape(B, H, S, W, Dh)
        logits = jnp.einsum("bhsd,bhswd->bhsw", q, kg) * scale
        logits = jnp.where(mask[None, None, :, :], logits, -1e9)
        attn = _softmax(logits, axis=-1)
        o = jnp.einsum("bhsw,bhswd->bhsd", attn, vg)
        return (lambda x, *d: x.transpose(*d))(o, 0, 2, 1, 3).reshape(B, S, D) @ wo

    def _B_ref(x, w_r, w_gate, w_up, w_down):
        B, S, D = x.shape
        C = 1
        r = x @ w_r
        idx = jnp.argsort(-r, axis=-1)[:, :C]
        idx_e = jnp.repeat(idx.reshape(B, C, 1), D, axis=2)
        x_sel = jnp.take_along_axis(x, idx_e, axis=1)
        g = _silu(x_sel @ w_gate)
        u = x_sel @ w_up
        y = (g * u) @ w_down
        r_sel = _sigmoid(jnp.take_along_axis(r, idx, axis=1))
        y = y * r_sel.reshape(B, C, 1)
        b_off = (jnp.arange(B) * S).reshape(B, 1)
        flat_idx = (idx + b_off).reshape(B * C)
        zero = (x * 0.0).reshape(B * S, D)
        upd = _scatter_add(zero, flat_idx, y.reshape(B * C, D), axis=0)
        return x + upd.reshape(B, S, D)

    x = A_x
    g = _sigmoid((x * gate_w).sum(-1, keepdims=True))
    a = _A_ref(x, A_wqkv, A_wo)
    b = _B_ref(x, B_w_r, B_w_gate, B_w_up, B_w_down)
    return g * a + (1 - g) * b
```

```python
import functools
import jax
import jax.numpy as jnp
from jax import lax
import jax.experimental.pallas as pl
import jax.experimental.pallas.tpu as pltpu

S, D, H, DH, F = 2048, 640, 32, 20, 1728
W, DIL = 8, 2
BS = 256
NB = S // BS
HALO = 16
NT = D // 128
FC = 64
LOG2E = 1.4426950408889634


def _interleave(*lists):
    items = []
    for li, l in enumerate(lists):
        for i, f in enumerate(l):
            items.append(((i + 0.5) / len(l), li, f))
    items.sort(key=lambda t: (t[0], t[1]))
    for _, _, f in items:
        f()


def _sigmoid(x):
    return 0.5 * jnp.tanh(0.5 * x) + 0.5


def _kernel(x_hbm, wqkv_hbm, wo_hbm, wg_hbm, wu_hbm, wd_hbm, wr_hbm, gw_hbm, out_hbm, wr_ref, gw_ref,
            x_v, w_v, wt_v, wo_v, wou_v, wg_v, wu_v, wd_v,
            qkv0, qkv1, o0, o1, o2, out_v, r_v, g_v, xs_v, y_v, best_v, besti_v, sems, csems, osems, idx_s):
    f32, bf16, u32, i32 = jnp.float32, jnp.bfloat16, jnp.uint32, jnp.int32
    qkvb = (qkv0, qkv1)
    ob = (o0, o1, o2)
    cp_w = [pltpu.make_async_copy(wqkv_hbm.at[pl.ds(c * 128, 128)], w_v.at[pl.ds(c * 128, 128)], csems.at[c])
            for c in range(NT)]
    cp_x0 = [pltpu.make_async_copy(x_hbm.at[pl.ds(0, BS), pl.ds(c * 128, 128)], x_v.at[c, pl.ds(0, BS)], csems.at[NT + c])
             for c in range(NT)]

    def x_copy(r0, n, sem):
        return [pltpu.make_async_copy(x_hbm.at[pl.ds(r0, n), pl.ds(c * 128, 128)], x_v.at[c, pl.ds(r0, n)], sems.at[sem])
                for c in range(NT)]
    cp_x1 = x_copy(BS, BS, 4)
    cp_x2 = x_copy(2 * BS, S - 2 * BS, 5)
    cp_wo = pltpu.make_async_copy(wo_hbm, wo_v, sems.at[6])
    def f_copy(a, b, r0, n, sem):
        return [pltpu.make_async_copy(a.at[pl.ds(r0, n), pl.ds(c * 128, 128)], b.at[c, pl.ds(r0, n)], sems.at[sem])
                for c in range(NT)]
    F0 = 9 * FC
    cp_fa = f_copy(wg_hbm, wg_v, 0, F0, 7) + f_copy(wu_hbm, wu_v, 0, F0, 7)
    cp_fb = f_copy(wg_hbm, wg_v, F0, F - F0, 8) + f_copy(wu_hbm, wu_v, F0, F - F0, 8)
    cp_fd = f_copy(wd_hbm, wd_v, 0, F, 9)
    for c in range(NT):
        cp_x0[c].start()
        cp_w[c].start()
    cp_vec = [pltpu.make_async_copy(wr_hbm, wr_ref, sems.at[1]), pltpu.make_async_copy(gw_hbm, gw_ref, sems.at[2])]
    for c in cp_vec + cp_x1 + [cp_wo]:
        c.start()
    qkv0[pl.ds(NT, NT), pl.ds(0, HALO), :] = jnp.zeros((NT, HALO, 128), f32)
    best_v[...] = jnp.full((8, 128), -jnp.inf, f32)
    besti_v[...] = jnp.zeros((8, 128), i32)
    for n in range(1, 16):
        idx_s[n] = 0
    z = idx_s[1]

    def prep_w(c):
        def tr(j):
            def f():
                t = w_v[c * 128:(c + 1) * 128, j * 128:(j + 1) * 128].T
                wt_v[c, pl.ds(j * 64, 64), :] = pltpu.bitcast(t, u32)
            return f
        return [tr(n) for n in range(3 * NT)]

    def prep_wo():
        def f(c):
            def g():
                wou_v[c, pl.ds(0, D // 2), :] = pltpu.bitcast(wo_v[:, c * 128:(c + 1) * 128], u32)
            return g
        return [f(c) for c in range(NT)]

    def perm_rows(ref, c, nmat):
        return jnp.concatenate([ref[c, pl.ds(p * 320 + e, H, stride=10), :]
                                for p in range(nmat) for e in range(DH // 2)], axis=0)

    def load_x(r0, n):
        return jnp.concatenate([x_v[c, pl.ds(r0, n), :] for c in range(NT)], axis=1)

    def row(ref):
        return ref[...].astype(f32).reshape(1, D)
    dn = (((1,), (1,)), ((), ()))
    qscale = DH ** -0.5 * LOG2E

    def a0_partial(c):
        st = {}
        def chunk(n):
            def f():
                if n == 0:
                    wch = pltpu.bitcast(perm_rows(wt_v, c, 3), bf16)
                    st['res'] = lax.dot_general(x_v[c, pl.ds(0, BS), :], wch, dn, preferred_element_type=f32)
                val = st['res'][:, n * 128:(n + 1) * 128]
                if c > 0:
                    val = val + qkv0[n, pl.ds(HALO, BS), :]
                if c == NT - 1 and n < NT:
                    val = val * qscale
                qkv0[n, pl.ds(HALO, BS), :] = val
            return f
        return [chunk(n) for n in range(3 * NT)]

    def stage_a(i):
        s = i % 2
        st = {}
        def chunk(n):
            def f():
                if n == 0:
                    wch = pltpu.bitcast(jnp.concatenate([perm_rows(wt_v, c, 3) for c in range(NT)], axis=1), bf16)
                    st['res'] = lax.dot_general(load_x(i * BS, BS), wch, dn, preferred_element_type=f32)
                val = st['res'][:, n * 128:(n + 1) * 128]
                if n < NT:
                    val = val * qscale
                qkvb[s][n, pl.ds(HALO, BS), :] = val
            return f
        return [chunk(n) for n in range(3 * NT)]

    def stage_r(i):
        def chunk(g):
            def f():
                r0 = i * BS + g * 64
                xf = load_x(r0, 64).astype(f32)
                r = jnp.sum(xf * row(wr_ref), axis=1, keepdims=True).astype(bf16).astype(f32)
                gate = _sigmoid(jnp.sum(xf * row(gw_ref), axis=1, keepdims=True))
                g_v[pl.ds(r0, 64), :] = jnp.broadcast_to(gate, (64, 128))
                b, bi = best_v[...], besti_v[...]
                for u in range(8):
                    ru = jnp.broadcast_to(r[u * 8:(u + 1) * 8], (8, 128))
                    up = ru > b
                    b = jnp.where(up, ru, b)
                    bi = jnp.where(up, r0 + u * 8, bi)
                best_v[...] = b
                besti_v[...] = bi
            return f
        return [chunk(g) for g in range(BS // 64)]

    lane = lax.broadcasted_iota(i32, (8, 128), 1)
    even = (lane & 1) == 0
    sub = lax.broadcasted_iota(i32, (8, 128), 0)

    def attn8(s, r, first):
        buf = qkvb[s]
        q = [buf[j, pl.ds(r + HALO, 8), :] for j in range(NT)]
        ss = []
        for w in range(W):
            t = None
            for j in range(NT):
                u = q[j] * buf[NT + j, pl.ds(z + r + HALO - DIL * w, 8), :]
                t = u if t is None else t + u
            t = t + pltpu.roll(t, 64, 1)
            t = t + jnp.where(even, pltpu.roll(t, 127, 1), pltpu.roll(t, 1, 1))
            if first and r - DIL * w < 0:
                t = jnp.where(sub + (r - DIL * w) >= 0, t, -1e9 * LOG2E)
            ss.append(t)
        m = functools.reduce(jnp.maximum, ss)
        ps = [jnp.exp2(t - m) for t in ss]
        l = functools.reduce(jnp.add, ps)
        inv = pl.reciprocal(l, approx=True)
        inv = inv * (2.0 - l * inv)
        accs = []
        for j in range(NT):
            acc = None
            for w in range(W):
                t = ps[w] * buf[2 * NT + j, pl.ds(z + r + HALO - DIL * w, 8), :]
                acc = t if acc is None else acc + t
            accs.append(acc * inv)
        return jnp.concatenate(accs, axis=1)

    def stage_b(i):
        s = i % 2
        def chunk(g):
            def f():
                a = attn8(s, g * 16, i == 0)
                b = attn8(s, g * 16 + 8, i == 0)
                ob[i % 3][pl.ds(g * 8, 8), :] = pltpu.bitcast(jnp.concatenate([a, b], axis=0).astype(bf16), u32)
                if g == 0 and i < NB - 1:
                    qkvb[1 - s][pl.ds(NT, 2 * NT), pl.ds(0, HALO), :] = qkvb[s][pl.ds(NT, 2 * NT), pl.ds(BS, HALO), :]
            return f
        return [chunk(g) for g in range(BS // 16)]

    def stage_c(i, j0=0, j1=NT):
        def f():
            r0 = i * BS
            g = g_v[pl.ds(r0, BS), :]
            a = jnp.dot(pltpu.bitcast(ob[i % 3][...], bf16), pltpu.bitcast(jnp.concatenate([perm_rows(wou_v, j, 1) for j in range(j0, j1)], axis=1), bf16), preferred_element_type=f32)
            for j in range(j0, j1):
                xb = x_v[j, pl.ds(r0, BS), :].astype(f32)
                out_v[pl.ds(r0, BS), j * 128:(j + 1) * 128] = (xb + g * (a[:, (j - j0) * 128:(j - j0 + 1) * 128] - xb)).astype(bf16)
        return [f]

    def out_copy(b):
        return pltpu.make_async_copy(out_v.at[pl.ds(b * BS, BS)], out_hbm.at[pl.ds(b * BS, BS)], osems.at[b])

    def ffn_sel():
        b, bi = best_v[...], besti_v[...] + sub
        mx = jnp.max(b)
        idx = jnp.min(jnp.where(b == mx, bi, S))
        idx = jnp.clip(idx, 0, S - 1)
        idx_s[0] = idx
        t0 = pl.multiple_of((idx // 16) * 16, 16)
        xf = load_x(t0, 16).astype(f32)
        hit = lax.broadcasted_iota(i32, (16, D), 0) == idx - t0
        xs = jnp.sum(jnp.where(hit, xf, 0.0), axis=0, keepdims=True)
        xs_v[...] = jnp.broadcast_to(xs, (8, D))
        g = _sigmoid(jnp.sum(xs * row(gw_ref), axis=1, keepdims=True))
        r_v[...] = jnp.where(hit, (1.0 - g) * _sigmoid(jnp.full((1, 1), mx, f32)), 0.0)

    def ffn():
        def chunk(g):
            def f():
                def mv(ref):
                    wv = jnp.concatenate([ref[c, pl.ds(g * FC, FC), :] for c in range(NT)], axis=1).astype(f32)
                    return jnp.sum(wv * xs_v[0:1, :], axis=1, keepdims=True)
                gg, uu = mv(wg_v), mv(wu_v)
                hh = gg * _sigmoid(gg) * uu
                hb = jnp.broadcast_to(hh, (FC, 128))
                for c in range(NT):
                    p = wd_v[c, pl.ds(g * FC, FC), :].astype(f32) * hb
                    y_v[pl.ds(g * 8, 8), c * 128:(c + 1) * 128] = jnp.sum(p.reshape(FC // 8, 8, 128), axis=0)
            return f
        return [chunk(g) for g in range(F // FC)]

    def patch(lo, hi, c0=0, c1=D):
        idx = idx_s[0]
        t0 = pl.multiple_of(jnp.clip((idx // 16) * 16, lo, hi - 16), 16)
        upd = jnp.where(jnp.logical_and(idx >= lo, idx < hi), r_v[:, c0:c1], 0.0)
        out_v[pl.ds(t0, 16), c0:c1] = (out_v[pl.ds(t0, 16), c0:c1].astype(f32) + upd).astype(bf16)

    def tile_copy():
        t0 = pl.multiple_of(jnp.minimum((idx_s[0] // 16) * 16, (NB - 4) * BS - 16), 16)
        return pltpu.make_async_copy(out_v.at[pl.ds(t0, 16)], out_hbm.at[pl.ds(t0, 16)], sems.at[0])

    def region(i, *lists):
        @pl.when(idx_s[2 + i] == 0)
        def _():
            for l in lists:
                _interleave(*l)

    cp_w[0].wait()
    _interleave(prep_w(0))
    for c in range(NT):
        cp_x0[c].wait()
        if c + 1 < NT:
            cp_w[c + 1].wait()
            _interleave(a0_partial(c), prep_w(c + 1))
        else:
            for cp in cp_x2 + cp_fa:
                cp.start()
            for cp in cp_vec + cp_x1:
                cp.wait()
            _interleave(a0_partial(c), stage_r(0) + stage_r(1))
    for j in range(2 * NT, 3 * NT):
        qkv0[j, pl.ds(0, HALO), :] = jnp.broadcast_to(qkv0[j, pl.ds(HALO, 1), :], (HALO, 128))
    cp_wo.wait()
    for c in cp_fb + cp_fd:
        c.start()
    region(1, (stage_a(1), stage_b(0), prep_wo()))
    for c in cp_x2:
        c.wait()

    up = ffn()
    extra = {2: stage_r(2) + stage_r(3) + stage_r(4) + stage_r(5)[:2], 3: stage_r(5)[2:] + stage_r(6) + stage_r(7) + [ffn_sel], 4: up[:9], 5: up[9:18], 6: up[18:]}
    for i in range(2, NB - 1):
        for c in {4: cp_fa + cp_fb + cp_fd}.get(i, []):
            c.wait()
        if i >= 3:
            out_copy(i - 3).start()
        region(i, (stage_c(i - 2),), (stage_a(i), stage_b(i - 1), extra[i]))

    def early_fix():
        r_v[...] = r_v[...] * jnp.sum(y_v[...], axis=0, keepdims=True)
        for b in range(NB - 4):
            out_copy(b).wait()
        patch(0, (NB - 3) * BS)
        tile_copy().start()
        out_copy(NB - 4).start()
    early_fix()
    region(NB - 1, (stage_a(NB - 1), stage_b(NB - 2)))

    def fin(b):
        def f():
            patch(b * BS, (b + 1) * BS)
            out_copy(b).start()
        return [f]
    region(NB, (stage_c(NB - 3) + fin(NB - 3) + stage_c(NB - 2) + fin(NB - 2), stage_b(NB - 1)))
    last = [pltpu.make_async_copy(out_v.at[pl.ds(S - BS, BS), pl.ds(a * 128, (b - a) * 128)],
                                  out_hbm.at[pl.ds(S - BS, BS), pl.ds(a * 128, (b - a) * 128)], csems.at[n])
            for n, (a, b) in enumerate(((0, 3), (3, 5)))]
    for n, (a, b) in enumerate(((0, 3), (3, 5))):
        _interleave(stage_c(NB - 1, a, b))
        patch(S - BS, S, a * 128, b * 128)
        last[n].start()
    for c in last:
        c.wait()
    for b in range(NB - 4, NB - 1):
        out_copy(b).wait()
    tile_copy().wait()


@jax.jit
def pallas_gated_mix__sliding_local_dilated__moe_arch_mod__prompt_kernel(
    A_x, A_wqkv, A_wo, B_x, B_w_r, B_w_gate, B_w_up, B_w_down, gate_w):
    f32, bf16, u32 = jnp.float32, jnp.bfloat16, jnp.uint32
    hbm = pl.BlockSpec(memory_space=pltpu.HBM)
    out = pl.pallas_call(
        _kernel,
        in_specs=[hbm] * 8,
        out_specs=hbm,
        out_shape=jax.ShapeDtypeStruct((S, D), bf16),
        scratch_shapes=[
            pltpu.VMEM((D,), bf16), pltpu.VMEM((D,), bf16),
            pltpu.VMEM((NT, S, 128), bf16), pltpu.VMEM((D, 3 * D), bf16),
            pltpu.VMEM((NT, 3 * D // 2 + 16, 128), u32),
            pltpu.VMEM((D, D), bf16), pltpu.VMEM((NT, D // 2 + 16, 128), u32),
            pltpu.VMEM((NT, F, 128), bf16), pltpu.VMEM((NT, F, 128), bf16), pltpu.VMEM((NT, F, 128), bf16),
            pltpu.VMEM((3 * NT, BS + HALO, 128), f32), pltpu.VMEM((3 * NT, BS + HALO, 128), f32),
            pltpu.VMEM((BS // 2, D), u32), pltpu.VMEM((BS // 2, D), u32), pltpu.VMEM((BS // 2, D), u32),
            pltpu.VMEM((S, D), bf16), pltpu.VMEM((16, D), f32), pltpu.VMEM((S, 128), f32),
            pltpu.VMEM((8, D), f32), pltpu.VMEM((F // FC * 8, D), f32),
            pltpu.VMEM((8, 128), f32), pltpu.VMEM((8, 128), jnp.int32),
            pltpu.SemaphoreType.DMA((10,)), pltpu.SemaphoreType.DMA((2 * NT,)), pltpu.SemaphoreType.DMA((NB,)),
            pltpu.SMEM((16,), jnp.int32),
        ],
        compiler_params=pltpu.CompilerParams(
            vmem_limit_bytes=100 * 1024 * 1024,
            flags={'XLA_TPU_EVENLY_DISTRIBUTE_CRITICAL_NODES': True}),
    )(A_x.reshape(S, D), A_wqkv, A_wo, B_w_gate.T, B_w_up.T, B_w_down, B_w_r, gate_w)
    return out.reshape(1, S, D)
```
